```python
import os as _os
_os.environ.setdefault("JAX_PLATFORMS", "cpu")
import jax
import jax.numpy as jnp

def _softmax(x, axis=-1):
    return jax.nn.softmax(x, axis=axis)
def _gelu(x):
    return jax.nn.gelu(x, approximate=True)
def _silu(x):
    return jax.nn.silu(x)
def _sigmoid(x):
    return jax.nn.sigmoid(x)
def _layernorm(x, axis=-1, eps=1e-5):
    m = jnp.mean(x, axis=axis, keepdims=True)
    v = jnp.var(x, axis=axis, keepdims=True)
    return (x - m) / jnp.sqrt(v + eps)
def _scatter_add(tgt, idx, src, axis=0):
    return tgt.at[idx].add(src)
def _segment_sum(src, seg, n):
    return jax.ops.segment_sum(src, seg, n)
class _Rng:
    def __init__(self, key):
        self._k = key
    def _next(self):
        self._k, sub = jax.random.split(self._k)
        return sub
    def normal(self, shape):
        return jax.random.normal(self._next(), shape, dtype=jnp.bfloat16)
    def randint(self, lo, hi, shape):
        return jax.random.randint(self._next(), shape, lo, hi, dtype=jnp.int32)
    def uniform(self, shape, lo=0.0, hi=1.0):
        return jax.random.uniform(self._next(), shape, jnp.bfloat16, lo, hi)
    def permutation(self, n):
        return jax.random.permutation(self._next(), n)


kernel_name = 'gated_mix__grouped_kv_mqa__swiglu_ffn__prompt'

def setup_inputs():
    _rng = _Rng(jax.random.key(int.from_bytes(__import__("os").urandom(4), "little")))
    _w = (lambda a: (lambda t: t.astype(jnp.bfloat16) if jnp.issubdtype(t.dtype, jnp.floating) else t)(jnp.asarray(a)))
    def _A_setup():
        B, S, D, H = 1, 2048, 512, 32
        Dh = D // H
        return {
            "x": _w((lambda *s: _rng.normal(s) * 0.05)(B, S, D)),
            "wq": _w((lambda *s: _rng.normal(s) * 0.4)(D, H * Dh)),
            "wk": _w((lambda *s: _rng.normal(s) * 0.4)(D, Dh)),
            "wv": _w((lambda *s: _rng.normal(s) * 0.05)(D, Dh)),
            "wo": _w((lambda *s: _rng.normal(s) * 0.05)(H * Dh, D)),
        }
    _A_in = _A_setup()

    def _B_setup():
        B, S, D, F = 1, 2048, 512, 1792
        return {
            "x": _w((lambda *s: _rng.normal(s) * 0.05)(B, S, D)),
            "w_gate": _w((lambda *s: _rng.normal(s) * 0.05)(D, F)),
            "w_up": _w((lambda *s: _rng.normal(s) * 0.05)(D, F)),
            "w_down": _w((lambda *s: _rng.normal(s) * 0.05)(F, D)),
        }
    _B_in = _B_setup()

    return {
        "A_x": _A_in["x"],
        "A_wq": _A_in["wq"],
        "A_wk": _A_in["wk"],
        "A_wv": _A_in["wv"],
        "A_wo": _A_in["wo"],
        "B_x": _B_in["x"],
        "B_w_gate": _B_in["w_gate"],
        "B_w_up": _B_in["w_up"],
        "B_w_down": _B_in["w_down"],
        "gate_w": _w((lambda *s: _rng.normal(s) * 0.05)(512) * 16.0),
    }

def reference(A_x, A_wq, A_wk, A_wv, A_wo, B_x, B_w_gate, B_w_up, B_w_down, gate_w):
    def _A_ref(x, wq, wk, wv, wo):
        B, S, D = x.shape
        H = 32
        Dh = D // H
        q = (lambda x, *d: x.transpose(*d))((x @ wq).reshape(B, S, H, Dh), 0, 2, 1, 3)
        k = x @ wk
        v = x @ wv
        scores = jnp.einsum("bhqd,bkd->bhqk", q, k) * (Dh ** -0.5)
        p = _softmax(scores, axis=-1)
        o = jnp.einsum("bhqk,bkd->bhqd", p, v)
        return (lambda x, *d: x.transpose(*d))(o, 0, 2, 1, 3).reshape(B, S, H * Dh) @ wo

    def _B_ref(x, w_gate, w_up, w_down):
        g = _silu(x @ w_gate)
        u = x @ w_up
        return (g * u) @ w_down

    x = A_x
    g = _sigmoid((x * gate_w).sum(-1, keepdims=True))
    a = _A_ref(x, A_wq, A_wk, A_wv, A_wo)
    b = _B_ref(x, B_w_gate, B_w_up, B_w_down)
    return g * a + (1 - g) * b
```

```python
import math

import jax
import jax.numpy as jnp
from jax import lax
import jax.experimental.pallas as pl
import jax.experimental.pallas.tpu as pltpu

S, D, H, DH, F = 2048, 512, 32, 16, 1792
TQ = 512
NQ = S // TQ
CK = 128
NC = S // CK
TC = 512
NX = S // TC
TM = 256
NM = S // TM
FC = 256
WROWS = H * DH + 2 * DH
KSCALE = (DH ** -0.5) * math.log2(math.e)

_F32 = jnp.float32
_BF16 = jnp.bfloat16


def _kernel(x_hbm, wq_hbm, wkt_ref, wvt_ref, wo_hbm, wg_hbm, wu_hbm, wd_hbm, gw_ref,
            out_hbm,
            x_v, wq_v, wo_v, wg_v, wu_v, wd_v, wt_v, qt_v, k_v, vt_v, ot_v, s_v, m_v,
            out_v, in_sems, out_sems):
    cp_wq = pltpu.make_async_copy(wq_hbm, wq_v, in_sems.at[0])
    cp_x = [pltpu.make_async_copy(x_hbm.at[pl.ds(c * TC, TC)], x_v.at[pl.ds(c * TC, TC)],
                                  in_sems.at[1 + c]) for c in range(NX)]
    cp_w = [pltpu.make_async_copy(src, dst, in_sems.at[1 + NX + i])
            for i, (src, dst) in enumerate(((wg_hbm, wg_v), (wu_hbm, wu_v), (wd_hbm, wd_v),
                                            (wo_hbm, wo_v)))]
    cp_wq.start()
    for cp in cp_x:
        cp.start()
    for cp in cp_w:
        cp.start()

    wt_v[H * DH:H * DH + DH, :] = wkt_ref[...]
    wt_v[H * DH + DH:WROWS, :] = wvt_ref[...]
    cp_wq.wait()
    wt_v[0:H * DH, :] = wq_v[...].T

    for c in range(NX):
        cp_x[c].wait()
        r = lax.dot_general(wt_v[...], x_v[c * TC:(c + 1) * TC, :],
                            (((1,), (1,)), ((), ())), preferred_element_type=_F32)
        qt_v[:, c * TC:(c + 1) * TC] = r[0:H * DH].astype(_BF16)
        kt = r[H * DH:H * DH + DH] * KSCALE
        k_v[c * TC:(c + 1) * TC, :] = kt.T.astype(_BF16)
        vt_v[:, c * TC:(c + 1) * TC] = r[H * DH + DH:WROWS].astype(_BF16)

    def q_tile(h, u):
        return qt_v[pl.ds(pl.multiple_of(h * DH, DH), DH), pl.ds(u * TQ, TQ)]

    def scores_chunk(u, qt, c, m):
        s = jnp.dot(k_v[c * CK:(c + 1) * CK, :], qt, preferred_element_type=_F32)
        s_v[u, c * CK:(c + 1) * CK, :] = s
        for r in range(CK // 8):
            sr = s[r * 8:(r + 1) * 8]
            m = sr if m is None else jnp.maximum(m, sr)
        return m

    def soft_chunk(u, c, m, l, acc):
        slabs = [None] * (CK // 16)
        for rr in reversed(range(CK // 16)):
            lo = c * CK + rr * 16
            p1 = jnp.exp2(s_v[u, lo + 8:lo + 16, :] - m)
            p0 = jnp.exp2(s_v[u, lo:lo + 8, :] - m)
            ps = p0 + p1
            l = ps if l is None else l + ps
            slabs[rr] = jnp.concatenate([p0, p1], axis=0)
        pb = jnp.concatenate(slabs, axis=0).astype(_BF16)
        o = jnp.dot(vt_v[:, c * CK:(c + 1) * CK], pb, preferred_element_type=_F32)
        return l, (o if acc is None else acc + o)

    def finish(h, u, l, acc):
        lt = jnp.sum(l, axis=0, keepdims=True)
        ot_v[pl.ds(pl.multiple_of(h * DH, DH), DH), pl.ds(u * TQ, TQ)] = (
            (acc / lt).astype(_BF16))

    def store_max(u, m8):
        m_v[u] = jnp.broadcast_to(jnp.max(m8, axis=0, keepdims=True), (8, TQ))

    def prologue(u, carry):
        u = pl.multiple_of(u, 1)
        qt = qt_v[0:DH, pl.ds(pl.multiple_of(u * TQ, TQ), TQ)]
        m8 = None
        for c in range(NC):
            m8 = scores_chunk(u, qt, c, m8)
        store_max(u, m8)
        return carry

    lax.fori_loop(0, NQ, prologue, 0)

    def body(h, carry):
        for u in range(NQ):
            qt = q_tile(h + 1, u)
            mb = m_v[u]
            m8 = None
            l = None
            acc = None
            for c in range(NC):
                l, acc = soft_chunk(u, c, mb, l, acc)
                m8 = scores_chunk(u, qt, c, m8)
            finish(h, u, l, acc)
            store_max(u, m8)
        return carry

    lax.fori_loop(0, H - 1, body, 0)

    def epilogue(u, carry):
        mb = m_v[u]
        l = None
        acc = None
        for c in range(NC):
            l, acc = soft_chunk(u, c, mb, l, acc)
        lt = jnp.sum(l, axis=0, keepdims=True)
        ot_v[(H - 1) * DH:H * DH, pl.ds(pl.multiple_of(u * TQ, TQ), TQ)] = (
            (acc / lt).astype(_BF16))
        return carry

    lax.fori_loop(0, NQ, epilogue, 0)

    for cp in cp_w:
        cp.wait()

    def out_copy(t):
        r0 = pl.multiple_of(t * TM, TM)
        return pltpu.make_async_copy(out_v.at[pl.ds(r0, TM)], out_hbm.at[pl.ds(r0, TM)],
                                     out_sems.at[t])

    def dense(t, carry):
        r0 = pl.multiple_of(t * TM, TM)
        x = x_v[pl.ds(r0, TM), :]
        xf = x.astype(_F32)
        gw = gw_ref[...].astype(_F32)
        z = xf[:, 0:128] * gw[0:1, :]
        for j in range(1, D // 128):
            z = z + xf[:, j * 128:(j + 1) * 128] * gw[j:j + 1, :]
        gate = jax.nn.sigmoid(jnp.sum(z, axis=-1, keepdims=True))
        b = None
        for f in range(F // FC):
            g = jnp.dot(x, wg_v[:, f * FC:(f + 1) * FC], preferred_element_type=_F32)
            uu = jnp.dot(x, wu_v[:, f * FC:(f + 1) * FC], preferred_element_type=_F32)
            hh = (g * jax.nn.sigmoid(g) * uu).astype(_BF16)
            d = jnp.dot(hh, wd_v[f * FC:(f + 1) * FC, :], preferred_element_type=_F32)
            b = d if b is None else b + d
        ot = ot_v[:, pl.ds(r0, TM)]
        a = lax.dot_general(ot, wo_v[...], (((0,), (0,)), ((), ())),
                            preferred_element_type=_F32)
        out_v[pl.ds(r0, TM), :] = (gate * a + (1.0 - gate) * b).astype(_BF16)
        out_copy(t).start()
        return carry

    lax.fori_loop(0, NM, dense, 0)

    for t in range(NM):
        out_copy(t).wait()


@jax.jit
def pallas_gated_mix__grouped_kv_mqa__swiglu_ffn__prompt_kernel(
    A_x: jax.Array,
    A_wq: jax.Array,
    A_wk: jax.Array,
    A_wv: jax.Array,
    A_wo: jax.Array,
    B_x: jax.Array,
    B_w_gate: jax.Array,
    B_w_up: jax.Array,
    B_w_down: jax.Array,
    gate_w: jax.Array,
):
    del B_x
    x = A_x.reshape(S, D)
    any_spec = pl.BlockSpec(memory_space=pl.ANY)
    vmem_spec = pl.BlockSpec(memory_space=pltpu.VMEM)
    out = pl.pallas_call(
        _kernel,
        out_shape=jax.ShapeDtypeStruct((S, D), _BF16),
        in_specs=[any_spec, any_spec, vmem_spec, vmem_spec, any_spec, any_spec, any_spec,
                  any_spec, vmem_spec],
        out_specs=any_spec,
        scratch_shapes=[
            pltpu.VMEM((S, D), _BF16),
            pltpu.VMEM((D, H * DH), _BF16),
            pltpu.VMEM((H * DH, D), _BF16),
            pltpu.VMEM((D, F), _BF16),
            pltpu.VMEM((D, F), _BF16),
            pltpu.VMEM((F, D), _BF16),
            pltpu.VMEM((WROWS, D), _BF16),
            pltpu.VMEM((H * DH, S), _BF16),
            pltpu.VMEM((S, DH), _BF16),
            pltpu.VMEM((DH, S), _BF16),
            pltpu.VMEM((H * DH, S), _BF16),
            pltpu.VMEM((NQ, S, TQ), _F32),
            pltpu.VMEM((NQ, 8, TQ), _F32),
            pltpu.VMEM((S, D), _BF16),
            pltpu.SemaphoreType.DMA((1 + NX + 4,)),
            pltpu.SemaphoreType.DMA((NM,)),
        ],
        compiler_params=pltpu.CompilerParams(vmem_limit_bytes=100 * 1024 * 1024),
    )(x, A_wq, A_wk.T, A_wv.T, A_wo, B_w_gate, B_w_up, B_w_down, gate_w.reshape(D // 128, 128))
    return out.reshape(1, S, D)
```

```python
import math

import jax
import jax.numpy as jnp
from jax import lax
import jax.experimental.pallas as pl
import jax.experimental.pallas.tpu as pltpu

S, D, H, DH, F = 2048, 512, 32, 16, 1792
TQ = 512
NQ = S // TQ
NT = S // 128
CK = 128
NC = S // CK
TC = 512
NX = S // TC
TM = 256
NM = S // TM
FC = 256
WROWS = H * DH + 2 * DH
KA = 2 * DH
QR = DH + 1
KSCALE = (DH ** -0.5) * math.log2(math.e)

MSL = [(c, g) for c in range(NC) for g in range(7, 0, -1)]
NMS = len(MSL)
LAG = 10
NCH = 2

L_LO = 2.0 ** -80
L_HI = 2.0 ** 60

_F32 = jnp.float32
_BF16 = jnp.bfloat16
_U32 = jnp.uint32


def _bf(v):
    return pltpu.bitcast(v, _BF16)


def _u32(v):
    return pltpu.bitcast(v, _U32)


def _kernel(x_hbm, wq_hbm, wkt_ref, wvt_ref, wo_hbm, wg_hbm, wu_hbm, wd_hbm, gw_ref,
            out_hbm,
            x_v, wq_v, wo_v, wg_v, wu_v, wd_v, wt_v, qt_v, kp_v, kn_v, kb_v, vt_v, kap_v,
            z_v, qb_a, qhi_a, qb_b, qhi_b, ot_v, s_v, out_v, in_sems, out_sems):
    cp_wq = pltpu.make_async_copy(wq_hbm, wq_v, in_sems.at[0])
    cp_x = [pltpu.make_async_copy(x_hbm.at[pl.ds(c * TC, TC)], x_v.at[pl.ds(c * TC, TC)],
                                  in_sems.at[1 + c]) for c in range(NX)]
    cp_w = [pltpu.make_async_copy(src, dst, in_sems.at[1 + NX + i])
            for i, (src, dst) in enumerate(((wg_hbm, wg_v), (wu_hbm, wu_v), (wd_hbm, wd_v),
                                            (wo_hbm, wo_v)))]
    cp_wq.start()
    for cp in cp_x:
        cp.start()
    for cp in cp_w:
        cp.start()

    z_v[...] = jnp.zeros((8, 128), jnp.int32)
    wt_v[0:DH, :] = wkt_ref[...]
    wt_v[DH:2 * DH, :] = wvt_ref[...]
    cp_wq.wait()
    wt_v[2 * DH:WROWS, :] = wq_v[...].T

    kmax = None
    for c in range(NX):
        cp_x[c].wait()
        r = lax.dot_general(wt_v[...], x_v[c * TC:(c + 1) * TC, :],
                            (((1,), (1,)), ((), ())), preferred_element_type=_F32)
        kt = (r[0:DH] * KSCALE).astype(_BF16).astype(_F32)
        for t in range(TC // 128):
            a = jnp.abs(kt[:, t * 128:(t + 1) * 128])
            kmax = a if kmax is None else jnp.maximum(kmax, a)
        vt_v[:, c * TC:(c + 1) * TC] = _u32(r[DH:2 * DH].astype(_BF16))
        kaug = jnp.concatenate([kt, jnp.full((DH, TC), -1.0, _F32)], axis=0).T
        kn_v[c * TC:(c + 1) * TC, :] = kaug[:, 0:DH].astype(_BF16)
        kpk = _u32(kaug.astype(_BF16))
        for cc in range(TC // CK):
            cg = c * (TC // CK) + cc
            for g in range(1, 8):
                i = cg * 7 + (7 - g)
                kp_v[i * 8:(i + 1) * 8, :] = kpk[cc * 64 + g * 8:cc * 64 + (g + 1) * 8]
            for gg in range(2):
                rows = kaug[cc * CK + gg * 8:cc * CK + (gg + 1) * 8]
                for d in range(DH):
                    kb_v[(cg * 2 + gg) * DH + d] = jnp.broadcast_to(rows[:, d:d + 1], (8, TQ))
        qt_v[:, c * TC:(c + 1) * TC] = _u32(r[2 * DH:WROWS].astype(_BF16))
    kap_v[...] = jnp.broadcast_to(jnp.max(kmax, axis=1, keepdims=True), (DH, 128))

    def prep_tile(h, slot, T):
        qb_ref, qhi_ref = (qb_a, qhi_a) if slot == 0 else (qb_b, qhi_b)
        qp = qt_v[pl.ds(pl.multiple_of(h * 8, 8), 8), T * 128:(T + 1) * 128]
        q = _bf(qp).astype(_F32)
        for d in range(DH):
            qb_ref[T * QR + d] = jnp.broadcast_to(q[d:d + 1, :], (8, 128))
        w = (jnp.abs(q) * kap_v[...]).astype(_BF16)
        qhi_ref[:, T * 128:(T + 1) * 128] = _u32(w)
        nb = -jnp.sum(w.astype(_F32), axis=0, keepdims=True)
        qb_ref[T * QR + DH] = jnp.broadcast_to(nb, (8, 128))

    for T in range(NT):
        prep_tile(0, 0, T)

    def head(h, carry, cur):
        lmin, lmax = carry
        qb_ref, qhi_ref = (qb_a, qhi_a) if cur == 0 else (qb_b, qhi_b)
        zi = z_v[...]
        zmask = zi != 0
        zf = pltpu.bitcast(zi, _F32)
        zf = jnp.concatenate([jnp.concatenate([zf] * 4, axis=1)] * 2, axis=0)
        hn = jnp.minimum(h + 1, H - 1)
        P = {}
        L = [None] * NQ
        ACC = [None] * NQ

        def q_aug(u):
            lo = qt_v[pl.ds(pl.multiple_of(h * 8, 8), 8), u * TQ:(u + 1) * TQ]
            hi = qhi_ref[:, u * TQ:(u + 1) * TQ]
            return _bf(jnp.concatenate([lo, hi], axis=0))

        def consume(u, c, g, s0, s1):
            p0 = jnp.exp2(s0)
            p1 = jnp.exp2(s1)
            t = p0 + p1
            L[u] = t if L[u] is None else L[u] + t
            P[(u, c, g)] = (p0, p1)

        def do_scores(u, i0, i1):
            s = jnp.dot(_bf(kp_v[i0 * 8:i1 * 8, :]), q_aug(u), preferred_element_type=_F32)
            for i in range(i0, i1):
                c, g = MSL[i]
                o = (i - i0) * 16
                consume(u, c, g, s[o:o + 8], s[o + 8:o + 16])

        def do_vpu(u, c):
            res = {}
            chain = []
            for t in range(4):
                base = (u * 4 + t) * QR
                for gg in range(2):
                    a = qb_ref[base + DH]
                    if len(chain) >= NCH:
                        a = jnp.where(zmask, chain[-NCH], a)
                    for d in range(DH):
                        a = a + (kb_v[(c * 2 + gg) * DH + d, :, t * 128:(t + 1) * 128]
                                 * qb_ref[base + d])
                    res[(t, gg)] = a
                    chain.append(a)
            consume(u, c, 0,
                    jnp.concatenate([res[(t, 0)] for t in range(4)], axis=1),
                    jnp.concatenate([res[(t, 1)] for t in range(4)], axis=1))

        def do_pv(u, c):
            do_vpu(u, c)
            ps = []
            for g in range(8):
                ps += list(P.pop((u, c, g)))
            pb = jnp.concatenate(ps, axis=0).astype(_BF16)
            o = jnp.dot(_bf(vt_v[:, c * CK:(c + 1) * CK]), pb, preferred_element_type=_F32)
            ACC[u] = (o + zf) if ACC[u] is None else ACC[u] + o
            if c == NC - 1:
                lt = jnp.sum(L[u], axis=0, keepdims=True)
                ot_v[pl.ds(pl.multiple_of(h * DH, DH), DH), u * TQ:(u + 1) * TQ] = (
                    (ACC[u] / lt).astype(_BF16))
                L[u] = lt
            if c % 4 == 1:
                prep_tile(hn, 1 - cur, u * 4 + c // 4)

        tot = NQ * NMS
        pv_at = {}
        for u in range(NQ):
            for c in range(NC):
                pos = min(u * NMS + c * 7 + 6 + LAG, tot)
                pv_at.setdefault(pos, []).append((u, c))
        start = 0
        for gi in range(tot + 1):
            u, i = divmod(gi, NMS)
            if gi < tot and (gi in pv_at or i == NMS - 1):
                do_scores(u, start, i + 1)
                start = (i + 1) % NMS
            for (uu, cc) in pv_at.get(gi, []):
                do_pv(uu, cc)
        for u in range(NQ):
            lmin = jnp.minimum(lmin, L[u])
            lmax = jnp.maximum(lmax, L[u])
        return lmin, lmax

    def body(h, carry):
        return lax.cond(h % 2 == 0, lambda: head(h, carry, 0), lambda: head(h, carry, 1))

    lmin, lmax = lax.fori_loop(
        0, H, body, (jnp.full((1, TQ), L_HI, _F32), jnp.full((1, TQ), L_LO, _F32)))
    safe = jnp.logical_and(lmin >= L_LO, lmax <= L_HI)
    n_unsafe = jnp.sum(jnp.where(safe, 0.0, 1.0))

    @pl.when(n_unsafe > 0.0)
    def _():
        def item(i, carry):
            h = i // NQ
            c0 = pl.multiple_of((i % NQ) * TQ, TQ)
            qt = _bf(qt_v[pl.ds(pl.multiple_of(h * 8, 8), 8), pl.ds(c0, TQ)])
            m8 = None
            for c in range(NC):
                s = jnp.dot(kn_v[c * CK:(c + 1) * CK, :], qt, preferred_element_type=_F32)
                s_v[c * CK:(c + 1) * CK, :] = s
                sm = jnp.max(s.reshape(CK // 8, 8, TQ), axis=0)
                m8 = sm if m8 is None else jnp.maximum(m8, sm)
            m = jnp.max(m8, axis=0, keepdims=True)

            def pv(c, st):
                l, acc = st
                r0 = pl.multiple_of(c * CK, CK)
                p = jnp.exp2(s_v[pl.ds(r0, CK), :] - m)
                l = l + jnp.sum(p.reshape(CK // 8, 8, TQ), axis=0)
                acc = acc + jnp.dot(_bf(vt_v[:, pl.ds(r0, CK)]), p.astype(_BF16),
                                    preferred_element_type=_F32)
                return l, acc

            l, acc = lax.fori_loop(0, NC, pv, (jnp.zeros((8, TQ), _F32),
                                               jnp.zeros((DH, TQ), _F32)))
            lt = jnp.sum(l, axis=0, keepdims=True)
            ot_v[pl.ds(pl.multiple_of(h * DH, DH), DH), pl.ds(c0, TQ)] = (
                (acc / lt).astype(_BF16))
            return carry

        lax.fori_loop(0, H * NQ, item, 0)

    for cp in cp_w:
        cp.wait()

    def out_copy(t):
        r0 = pl.multiple_of(t * TM, TM)
        return pltpu.make_async_copy(out_v.at[pl.ds(r0, TM)], out_hbm.at[pl.ds(r0, TM)],
                                     out_sems.at[t])

    def dense(t, carry):
        r0 = pl.multiple_of(t * TM, TM)
        x = x_v[pl.ds(r0, TM), :]
        xf = x.astype(_F32)
        gw = gw_ref[...].astype(_F32)
        z = xf[:, 0:128] * gw[0:1, :]
        for j in range(1, D // 128):
            z = z + xf[:, j * 128:(j + 1) * 128] * gw[j:j + 1, :]
        gate = jax.nn.sigmoid(jnp.sum(z, axis=-1, keepdims=True))
        b = None
        for f in range(F // FC):
            g = jnp.dot(x, wg_v[:, f * FC:(f + 1) * FC], preferred_element_type=_F32)
            uu = jnp.dot(x, wu_v[:, f * FC:(f + 1) * FC], preferred_element_type=_F32)
            hh = (g * jax.nn.sigmoid(g) * uu).astype(_BF16)
            d = jnp.dot(hh, wd_v[f * FC:(f + 1) * FC, :], preferred_element_type=_F32)
            b = d if b is None else b + d
        ot = ot_v[:, pl.ds(r0, TM)]
        a = lax.dot_general(ot, wo_v[...], (((0,), (0,)), ((), ())),
                            preferred_element_type=_F32)
        out_v[pl.ds(r0, TM), :] = (gate * a + (1.0 - gate) * b).astype(_BF16)
        out_copy(t).start()
        return carry

    lax.fori_loop(0, NM, dense, 0)

    for t in range(NM):
        out_copy(t).wait()


@jax.jit
def pallas_gated_mix__grouped_kv_mqa__swiglu_ffn__prompt_kernel(
    A_x: jax.Array,
    A_wq: jax.Array,
    A_wk: jax.Array,
    A_wv: jax.Array,
    A_wo: jax.Array,
    B_x: jax.Array,
    B_w_gate: jax.Array,
    B_w_up: jax.Array,
    B_w_down: jax.Array,
    gate_w: jax.Array,
):
    del B_x
    x = A_x.reshape(S, D)
    any_spec = pl.BlockSpec(memory_space=pl.ANY)
    vmem_spec = pl.BlockSpec(memory_space=pltpu.VMEM)
    out = pl.pallas_call(
        _kernel,
        out_shape=jax.ShapeDtypeStruct((S, D), _BF16),
        in_specs=[any_spec, any_spec, vmem_spec, vmem_spec, any_spec, any_spec, any_spec,
                  any_spec, vmem_spec],
        out_specs=any_spec,
        scratch_shapes=[
            pltpu.VMEM((S, D), _BF16),
            pltpu.VMEM((D, H * DH), _BF16),
            pltpu.VMEM((H * DH, D), _BF16),
            pltpu.VMEM((D, F), _BF16),
            pltpu.VMEM((D, F), _BF16),
            pltpu.VMEM((F, D), _BF16),
            pltpu.VMEM((WROWS, D), _BF16),
            pltpu.VMEM((H * DH // 2, S), _U32),
            pltpu.VMEM((NMS * 8, KA), _U32),
            pltpu.VMEM((S, DH), _BF16),
            pltpu.VMEM((NC * 2 * DH, 8, TQ), _F32),
            pltpu.VMEM((DH // 2, S), _U32),
            pltpu.VMEM((DH, 128), _F32),
            pltpu.VMEM((8, 128), jnp.int32),
            pltpu.VMEM((NT * QR, 8, 128), _F32),
            pltpu.VMEM((8, S), _U32),
            pltpu.VMEM((NT * QR, 8, 128), _F32),
            pltpu.VMEM((8, S), _U32),
            pltpu.VMEM((H * DH, S), _BF16),
            pltpu.VMEM((S, TQ), _F32),
            pltpu.VMEM((S, D), _BF16),
            pltpu.SemaphoreType.DMA((1 + NX + 4,)),
            pltpu.SemaphoreType.DMA((NM,)),
        ],
        compiler_params=pltpu.CompilerParams(vmem_limit_bytes=100 * 1024 * 1024),
    )(x, A_wq, A_wk.T, A_wv.T, A_wo, B_w_gate, B_w_up, B_w_down, gate_w.reshape(D // 128, 128))
    return out.reshape(1, S, D)
```

```python
import math

import jax
import jax.numpy as jnp
from jax import lax
import jax.experimental.pallas as pl
import jax.experimental.pallas.tpu as pltpu

S, D, H, DH, F = 2048, 512, 32, 16, 1792
TQ = 512
NQ = S // TQ
NT = S // 128
CK = 128
NC = S // CK
TC = 512
NX = S // TC
X_WAIT = (0, 1, 2, 2)
TM = 256
NM = S // TM
FC = 256
WROWS = H * DH + 2 * DH
KA = 2 * DH
QR = DH + 1
KSCALE = (DH ** -0.5) * math.log2(math.e)

MPC = 7
MSL = [(c, g) for c in range(NC) for g in range(MPC, 0, -1)]
NMS = len(MSL)
HB = 4
NW = HB * NQ
LAG = 10
NCH = 2
ANCHOR_LAST = 17
ANCHOR_CARRY = 17
ANCHOR_TAIL_PREP = (7, 6, 5, 4)

L_LO = 2.0 ** -80
L_HI = 2.0 ** 60

_F32 = jnp.float32
_BF16 = jnp.bfloat16
_U32 = jnp.uint32


def _bf(v):
    return pltpu.bitcast(v, _BF16)


def _u32(v):
    return pltpu.bitcast(v, _U32)


def _kernel(x_hbm, wq_hbm, wkt_hbm, wvt_hbm, wo_hbm, wg_hbm, wu_hbm, wd_hbm, gw_hbm,
            out_hbm,
            x_v, wq_v, wo_v, wg_v, wu_v, wd_v, gw_v, wt_v, qt_v, kp_v, kn_v, kb_v, vt_v,
            kap_v, z_v, pc_v, acc_v, l_v, ot_v, s_v, out_v, in_sems, out_sems, *bufs):
    qb_bufs, qhi_bufs = bufs[:HB], bufs[HB:]

    cp_wq = pltpu.make_async_copy(wq_hbm, wq_v, in_sems.at[0])
    cp_wk = pltpu.make_async_copy(wkt_hbm, wt_v.at[pl.ds(0, DH)], in_sems.at[1])
    cp_wv = pltpu.make_async_copy(wvt_hbm, wt_v.at[pl.ds(DH, DH)], in_sems.at[2])
    cp_x = [pltpu.make_async_copy(x_hbm.at[pl.ds(c * TC, TC)], x_v.at[pl.ds(c * TC, TC)],
                                  in_sems.at[3 + c]) for c in range(NX)]
    cp_w = [pltpu.make_async_copy(src, dst, in_sems.at[3 + NX + i])
            for i, (src, dst) in enumerate(((gw_hbm, gw_v), (wg_hbm, wg_v), (wu_hbm, wu_v),
                                            (wd_hbm, wd_v), (wo_hbm, wo_v)))]
    for cp in [cp_wq, cp_x[0], cp_wk, cp_wv] + cp_x[1:] + cp_w:
        cp.start()

    z_v[...] = jnp.zeros((8, 128), jnp.int32)
    pc_v[...] = jnp.zeros((2, CK // 2, TQ), _U32)
    acc_v[...] = jnp.zeros((DH, TQ), _F32)
    l_v[...] = jnp.ones((8, TQ), _F32)
    cp_wq.wait()
    wt_v[2 * DH:WROWS, :] = wq_v[...].T
    cp_wk.wait()
    cp_wv.wait()

    def bcast_rows(q, slot, T):
        for d in range(DH):
            qb_bufs[slot][T * QR + d] = jnp.broadcast_to(q[d:d + 1, :], (8, 128))

    def shift_rows(q, slot, T):
        w = (jnp.abs(q) * kap_v[...]).astype(_BF16)
        qhi_bufs[slot][:, T * 128:(T + 1) * 128] = _u32(w)
        nb = -jnp.sum(w.astype(_F32), axis=0, keepdims=True)
        qb_bufs[slot][T * QR + DH] = jnp.broadcast_to(nb, (8, 128))

    kmax = None
    for c in range(NX):
        for cc in range(NX):
            if X_WAIT[cc] == c:
                cp_x[cc].wait()
        r = lax.dot_general(wt_v[...], x_v[c * TC:(c + 1) * TC, :],
                            (((1,), (1,)), ((), ())), preferred_element_type=_F32)
        for t in range(TC // 128):
            T = c * (TC // 128) + t
            rt = r[:, t * 128:(t + 1) * 128]
            kt = (rt[0:DH] * KSCALE).astype(_BF16).astype(_F32)
            a = jnp.abs(kt)
            kmax = a if kmax is None else jnp.maximum(kmax, a)
            vt_v[:, T * 128:(T + 1) * 128] = _u32(rt[DH:2 * DH].astype(_BF16))
            kaug = jnp.concatenate([kt, jnp.full((DH, 128), -1.0, _F32)], axis=0).T
            kn_v[T * 128:(T + 1) * 128, :] = kaug[:, 0:DH].astype(_BF16)
            for g in range(MPC, 0, -1):
                i = T * MPC + (MPC - g)
                kp_v[i * 8:(i + 1) * 8, :] = _u32(kaug[g * 16:(g + 1) * 16].astype(_BF16))
            for gg in range(2):
                rows = kaug[gg * 8:(gg + 1) * 8]
                for d in range(DH):
                    kb_v[(T * 2 + gg) * DH + d] = jnp.broadcast_to(rows[:, d:d + 1], (8, TQ))
            qtile = rt[2 * DH:WROWS].astype(_BF16)
            qt_v[:, T * 128:(T + 1) * 128] = _u32(qtile)
            for slot in range(HB):
                bcast_rows(qtile[slot * DH:(slot + 1) * DH].astype(_F32), slot, T)
    kap_v[...] = jnp.broadcast_to(jnp.max(kmax, axis=1, keepdims=True), (DH, 128))
    for slot in range(HB):
        for T in range(NT):
            shift_rows(_bf(qt_v[slot * 8:(slot + 1) * 8, T * 128:(T + 1) * 128]).astype(_F32),
                       slot, T)

    def finish(hrow, u, l, acc):
        lt = jnp.sum(l, axis=0, keepdims=True)
        r0 = hrow * DH if isinstance(hrow, int) else pl.multiple_of(hrow * DH, DH)
        ot_v[pl.ds(r0, DH), u * TQ:(u + 1) * TQ] = (acc / lt).astype(_BF16)
        return lt

    def deferred_pv(j, acc):
        c = NC - 2 + j
        o = jnp.dot(_bf(vt_v[:, c * CK:(c + 1) * CK]), _bf(pc_v[j]),
                    preferred_element_type=_F32)
        return (acc_v[...] if acc is None else acc) + o

    def body(j, carry):
        lmin, lmax = carry
        h0 = j * HB
        zi = z_v[...]
        never = zi != 0
        zf = pltpu.bitcast(zi, _F32)
        zf = jnp.concatenate([jnp.concatenate([zf] * 4, axis=1)] * 2, axis=0)
        P = {}
        SC = {}
        L = [None] * NW
        ACC = [None] * NW
        prev = {}

        def pv_pos(w, c):
            return w * NMS + c * MPC + MPC - 1 + LAG

        def q_aug(w):
            hb, u = divmod(w, NQ)
            lo = qt_v[pl.ds(pl.multiple_of((h0 + hb) * 8, 8), 8), u * TQ:(u + 1) * TQ]
            hi = qhi_bufs[hb][:, u * TQ:(u + 1) * TQ]
            return _bf(jnp.concatenate([lo, hi], axis=0))

        def consume(w, c, g, s0, s1):
            p0 = jnp.exp2(s0)
            p1 = jnp.exp2(s1)
            t = p0 + p1
            L[w] = t if L[w] is None else L[w] + t
            P[(w, c, g)] = (p0, p1)

        def mxu_scores(w, i0, i1):
            s = jnp.dot(_bf(kp_v[i0 * 8:i1 * 8, :]), q_aug(w), preferred_element_type=_F32)
            for i in range(i0, i1):
                o = (i - i0) * 16
                consume(w, *MSL[i], s[o:o + 8], s[o + 8:o + 16])
                SC[w * NMS + i] = s[o:o + 8, 0:128]

        def vpu_scores(w, c, anchor):
            hb, u = divmod(w, NQ)
            qb_ref = qb_bufs[hb]
            res = {}
            chain = [] if anchor is None else [anchor] * NCH
            for t in range(4):
                base = (u * 4 + t) * QR
                for gg in range(2):
                    a = qb_ref[base + DH]
                    if len(chain) >= NCH:
                        a = jnp.where(never, chain[-NCH], a)
                    for d in range(DH):
                        a = a + (kb_v[(c * 2 + gg) * DH + d, :, t * 128:(t + 1) * 128]
                                 * qb_ref[base + d])
                    res[(t, gg)] = a
                    chain.append(a)
            consume(w, c, 0,
                    jnp.concatenate([res[(t, 0)] for t in range(4)], axis=1),
                    jnp.concatenate([res[(t, 1)] for t in range(4)], axis=1))

        def p_tile(w, c, anchor=None):
            vpu_scores(w, c, anchor)
            ps = []
            for g in range(8):
                ps += list(P.pop((w, c, g)))
            return jnp.concatenate(ps, axis=0).astype(_BF16)

        def refill(w, k, anchor):
            hb, u = divmod(w, NQ)
            T = u * 4 + k
            hn = jnp.minimum(h0 + hb + HB, H - 1)
            qp = qt_v[pl.ds(pl.multiple_of(hn * 8, 8), 8), T * 128:(T + 1) * 128]
            q = _bf(jnp.where(never, _u32(anchor), qp)).astype(_F32)
            bcast_rows(q, hb, T)
            shift_rows(q, hb, T)

        def do_pv(w, c):
            if w < 0:
                prev["acc"] = deferred_pv(c - (NC - 2), prev.get("acc"))
                if c == NC - 1:
                    prev["lt"] = finish(h0, NQ - 1, l_v[...], prev["acc"])
                return
            anchor = SC[pv_pos(w, c) - ANCHOR_LAST] if c == NC - 1 else None
            o = jnp.dot(_bf(vt_v[:, c * CK:(c + 1) * CK]), p_tile(w, c, anchor),
                        preferred_element_type=_F32)
            ACC[w] = (o + zf) if ACC[w] is None else ACC[w] + o
            if c == NC - 1:
                L[w] = finish(h0 + w // NQ + 1, w % NQ, L[w], ACC[w])
            if c % 4 == 1 and w > 0:
                refill(w - 1, c // 4, SC[pv_pos(w, c) - LAG])

        tot = NW * NMS
        pv_at = {}
        for w in range(-1, NW):
            for c in range(NC):
                if 0 <= pv_pos(w, c) < tot:
                    pv_at[pv_pos(w, c)] = (w, c)
        start = 0
        for gi in range(tot):
            w, i = divmod(gi, NMS)
            if gi in pv_at or i == NMS - 1:
                mxu_scores(w, start, i + 1)
                start = (i + 1) % NMS
            if gi in pv_at:
                do_pv(*pv_at[gi])
        for k in range(2):
            c = NC - 2 + k
            anchor = SC[pv_pos(NW - 1, c) - LAG - ANCHOR_CARRY]
            pc_v[k] = _u32(p_tile(NW - 1, c, anchor))
        acc_v[...] = ACC[NW - 1]
        l_v[...] = L[NW - 1]
        for k in range(4):
            refill(NW - 1, k, SC[tot - ANCHOR_TAIL_PREP[k]])
        for lt in [prev["lt"]] + L[:NW - 1]:
            lmin = jnp.minimum(lmin, lt)
            lmax = jnp.maximum(lmax, lt)
        return lmin, lmax

    lmin, lmax = lax.fori_loop(
        0, H // HB, body, (jnp.full((1, TQ), L_HI, _F32), jnp.full((1, TQ), L_LO, _F32)))
    lt = finish(H, NQ - 1, l_v[...], deferred_pv(1, deferred_pv(0, None)))
    lmin = jnp.minimum(lmin, lt)
    lmax = jnp.maximum(lmax, lt)
    safe = jnp.logical_and(lmin >= L_LO, lmax <= L_HI)
    n_unsafe = jnp.sum(jnp.where(safe, 0.0, 1.0))

    @pl.when(n_unsafe > 0.0)
    def _():
        def item(i, carry):
            h = i // NQ
            c0 = pl.multiple_of((i % NQ) * TQ, TQ)
            qt = _bf(qt_v[pl.ds(pl.multiple_of(h * 8, 8), 8), pl.ds(c0, TQ)])
            m8 = None
            for c in range(NC):
                s = jnp.dot(kn_v[c * CK:(c + 1) * CK, :], qt, preferred_element_type=_F32)
                s_v[c * CK:(c + 1) * CK, :] = s
                sm = jnp.max(s.reshape(CK // 8, 8, TQ), axis=0)
                m8 = sm if m8 is None else jnp.maximum(m8, sm)
            m = jnp.max(m8, axis=0, keepdims=True)

            def pv(c, st):
                l, acc = st
                r0 = pl.multiple_of(c * CK, CK)
                p = jnp.exp2(s_v[pl.ds(r0, CK), :] - m)
                l = l + jnp.sum(p.reshape(CK // 8, 8, TQ), axis=0)
                acc = acc + jnp.dot(_bf(vt_v[:, pl.ds(r0, CK)]), p.astype(_BF16),
                                    preferred_element_type=_F32)
                return l, acc

            l, acc = lax.fori_loop(0, NC, pv, (jnp.zeros((8, TQ), _F32),
                                               jnp.zeros((DH, TQ), _F32)))
            lt = jnp.sum(l, axis=0, keepdims=True)
            ot_v[pl.ds(pl.multiple_of((h + 1) * DH, DH), DH), pl.ds(c0, TQ)] = (
                (acc / lt).astype(_BF16))
            return carry

        lax.fori_loop(0, H * NQ, item, 0)

    for cp in cp_w:
        cp.wait()

    def out_copy(t):
        r0 = t * TM if isinstance(t, int) else pl.multiple_of(t * TM, TM)
        return pltpu.make_async_copy(out_v.at[pl.ds(r0, TM)], out_hbm.at[pl.ds(r0, TM)],
                                     out_sems.at[t])

    def dense(t, carry):
        r0 = pl.multiple_of(t * TM, TM)
        x = x_v[pl.ds(r0, TM), :]
        xf = x.astype(_F32)
        gw = gw_v[...].astype(_F32)
        z = xf[:, 0:128] * gw[0:1, :]
        for j in range(1, D // 128):
            z = z + xf[:, j * 128:(j + 1) * 128] * gw[j:j + 1, :]
        gate = jax.nn.sigmoid(jnp.sum(z, axis=-1, keepdims=True))
        b = None
        for f in range(F // FC):
            g = jnp.dot(x, wg_v[:, f * FC:(f + 1) * FC], preferred_element_type=_F32)
            uu = jnp.dot(x, wu_v[:, f * FC:(f + 1) * FC], preferred_element_type=_F32)
            hh = (g * jax.nn.sigmoid(g) * uu).astype(_BF16)
            d = jnp.dot(hh, wd_v[f * FC:(f + 1) * FC, :], preferred_element_type=_F32)
            b = d if b is None else b + d
        ot = ot_v[DH:(H + 1) * DH, pl.ds(r0, TM)]
        a = lax.dot_general(ot, wo_v[...], (((0,), (0,)), ((), ())),
                            preferred_element_type=_F32)
        out_v[pl.ds(r0, TM), :] = (gate * a + (1.0 - gate) * b).astype(_BF16)
        out_copy(t).start()
        return carry

    lax.fori_loop(0, NM, dense, 0)

    for t in range(NM):
        out_copy(t).wait()


@jax.jit
def pallas_gated_mix__grouped_kv_mqa__swiglu_ffn__prompt_kernel(
    A_x: jax.Array,
    A_wq: jax.Array,
    A_wk: jax.Array,
    A_wv: jax.Array,
    A_wo: jax.Array,
    B_x: jax.Array,
    B_w_gate: jax.Array,
    B_w_up: jax.Array,
    B_w_down: jax.Array,
    gate_w: jax.Array,
):
    del B_x
    any_spec = pl.BlockSpec(memory_space=pl.ANY)
    out = pl.pallas_call(
        _kernel,
        out_shape=jax.ShapeDtypeStruct((S, D), _BF16),
        in_specs=[any_spec] * 9,
        out_specs=any_spec,
        scratch_shapes=[
            pltpu.VMEM((S, D), _BF16),
            pltpu.VMEM((D, H * DH), _BF16),
            pltpu.VMEM((H * DH, D), _BF16),
            pltpu.VMEM((D, F), _BF16),
            pltpu.VMEM((D, F), _BF16),
            pltpu.VMEM((F, D), _BF16),
            pltpu.VMEM((D // 128, 128), _BF16),
            pltpu.VMEM((WROWS, D), _BF16),
            pltpu.VMEM((H * DH // 2, S), _U32),
            pltpu.VMEM((NMS * 8, KA), _U32),
            pltpu.VMEM((S, DH), _BF16),
            pltpu.VMEM((NC * 2 * DH, 8, TQ), _F32),
            pltpu.VMEM((DH // 2, S), _U32),
            pltpu.VMEM((DH, 128), _F32),
            pltpu.VMEM((8, 128), jnp.int32),
            pltpu.VMEM((2, CK // 2, TQ), _U32),
            pltpu.VMEM((DH, TQ), _F32),
            pltpu.VMEM((8, TQ), _F32),
            pltpu.VMEM(((H + 1) * DH, S), _BF16),
            pltpu.VMEM((S, TQ), _F32),
            pltpu.VMEM((S, D), _BF16),
            pltpu.SemaphoreType.DMA((3 + NX + 5,)),
            pltpu.SemaphoreType.DMA((NM,)),
        ] + [pltpu.VMEM((NT * QR, 8, 128), _F32)] * HB + [pltpu.VMEM((8, S), _U32)] * HB,
        compiler_params=pltpu.CompilerParams(vmem_limit_bytes=100 * 1024 * 1024),
    )(A_x.reshape(S, D), A_wq, A_wk.T, A_wv.T, A_wo, B_w_gate, B_w_up, B_w_down,
      gate_w.reshape(D // 128, 128))
    return out.reshape(1, S, D)
```

```python
import math

import jax
import jax.numpy as jnp
from jax import lax
import jax.experimental.pallas as pl
import jax.experimental.pallas.tpu as pltpu

S, D, H, DH, F = 2048, 512, 32, 16, 1792
TQ = 512
NQ = S // TQ
NT = S // 128
CK = 128
NC = S // CK
TC = 512
NX = S // TC
TM = 512
NM = S // TM
RM = S // H
NF = F // 128
WROWS = H * DH + 2 * DH
KA = 2 * DH
QR = DH + 1
KSCALE = (DH ** -0.5) * math.log2(math.e)

NVS = [2 if c in (0, 3, 8) else 1 for c in range(NC)]
VB = [sum(NVS[:c]) for c in range(NC + 1)]
MSL = [(c, g) for c in range(NC) for g in range(7, NVS[c] - 1, -1)]
NMS = len(MSL)
LASTS = [max(i for i, cg in enumerate(MSL) if cg[0] == c) for c in range(NC)]
HB = 4
NW = HB * NQ
LAG = 10
FFN_AFTER = {2: 2, 7: 2, 15: 3}
REFILL_AT = (1, 5, 9, 13)
ANCHOR_LAST = 16
ANCHOR_CARRY = 21
ANCHOR_TAIL_REFILL = (7, 6, 5, 4)
WG_REPACK = (0, 8, NF)

L_LO = 2.0 ** -80
L_HI = 2.0 ** 60

_F32 = jnp.float32
_BF16 = jnp.bfloat16
_U32 = jnp.uint32


def _bf(v):
    return pltpu.bitcast(v, _BF16)


def _u32(v):
    return pltpu.bitcast(v, _U32)


def _rep(v, n=2):
    return jnp.concatenate([v] * n, axis=0)


def _kernel(x_hbm, wq_hbm, wkt_hbm, wvt_hbm, wo_hbm, wg_hbm, wu_hbm, wd_hbm, gw_hbm,
            out_hbm,
            x_v, wq_v, wo_v, wg_v, wu_v, wd_v, gw_v, wgp_v, wup_v, wt_v, qt_v, kp_v, kn_v,
            kb_v, vt_v, kap_v, z_v, pc_v, acc_v, l_v, ot_v, h_v, s_v, out_v,
            in_sems, out_sems, *bufs):
    qb_bufs, qhi_bufs = bufs[:HB], bufs[HB:]

    def load(i, src, dst):
        return pltpu.make_async_copy(src, dst, in_sems.at[i])

    cp_x = [load(c, x_hbm.at[pl.ds(c * TC, TC)], x_v.at[pl.ds(c * TC, TC)]) for c in range(NX)]
    cp_wq = load(NX, wq_hbm, wq_v)
    cp_wk = load(NX + 1, wkt_hbm, wt_v.at[pl.ds(0, DH)])
    cp_wv = load(NX + 2, wvt_hbm, wt_v.at[pl.ds(DH, DH)])
    cp_wg = load(NX + 3, wg_hbm, wg_v)
    cp_wu = load(NX + 4, wu_hbm, wu_v)
    cp_gw = load(NX + 5, gw_hbm, gw_v)
    cp_wd = load(NX + 6, wd_hbm, wd_v)
    cp_wo = load(NX + 7, wo_hbm, wo_v)
    for cp in (cp_wq, cp_x[0], cp_wk, cp_wv, cp_x[1], cp_x[2], cp_wg, cp_x[3], cp_wu, cp_gw,
               cp_wd, cp_wo):
        cp.start()

    z_v[...] = jnp.zeros((8, 128), jnp.int32)
    pc_v[...] = jnp.zeros((2, CK // 2, TQ), _U32)
    acc_v[...] = jnp.zeros((DH, TQ), _F32)
    l_v[...] = jnp.ones((8, TQ), _F32)
    cp_wq.wait()
    wt_v[2 * DH:WROWS, :] = wq_v[...].T
    cp_wk.wait()
    cp_wv.wait()

    def bcast_rows(q, slot, T):
        for d in range(DH):
            qb_bufs[slot][T * QR + d] = jnp.broadcast_to(q[d:d + 1, :], (8, 128))

    def shift_rows(q, slot, T):
        w = (jnp.abs(q) * kap_v[...]).astype(_BF16)
        qhi_bufs[slot][:, T * 128:(T + 1) * 128] = _u32(w)
        nb = -jnp.sum(w.astype(_F32), axis=0, keepdims=True)
        qb_bufs[slot][T * QR + DH] = jnp.broadcast_to(nb, (8, 128))

    kmax = None
    for c in range(NX):
        cp_x[c].wait()
        if c == NX - 1:
            cp_wg.wait()
        r = lax.dot_general(wt_v[...], x_v[c * TC:(c + 1) * TC, :],
                            (((1,), (1,)), ((), ())), preferred_element_type=_F32)
        for t in range(TC // 128):
            T = c * (TC // 128) + t
            rt = r[:, t * 128:(t + 1) * 128]
            kt = (rt[0:DH] * KSCALE).astype(_BF16).astype(_F32)
            a = jnp.abs(kt)
            kmax = a if kmax is None else jnp.maximum(kmax, a)
            vt_v[:, T * 128:(T + 1) * 128] = _u32(rt[DH:2 * DH].astype(_BF16))
            kaug = jnp.concatenate([kt, jnp.full((DH, 128), -1.0, _F32)], axis=0).T
            kn_v[T * 128:(T + 1) * 128, :] = kaug[:, 0:DH].astype(_BF16)
            for i, (cc, g) in enumerate(MSL):
                if cc == T:
                    kp_v[i * 8:(i + 1) * 8, :] = _u32(kaug[g * 16:(g + 1) * 16].astype(_BF16))
            for g in range(NVS[T]):
                for d in range(DH):
                    kb_v[(VB[T] + g) * DH + d] = jnp.broadcast_to(
                        kaug[g * 16:(g + 1) * 16, d:d + 1], (16, TQ))
            if c == NX - 1 and t < len(WG_REPACK) - 1:
                f0, f1 = WG_REPACK[t], WG_REPACK[t + 1]
                for f in range(f0, f1):
                    row = (((f - f0) * WROWS) // (f1 - f0)) // 8 * 8
                    wgp_v[:, f * 128:(f + 1) * 128] = jnp.where(
                        _rep(z_v[...], D // 16) != 0, _rep(_u32(rt[row:row + 8]), D // 16),
                        _u32(wg_v[:, f * 128:(f + 1) * 128]))
            qtile = rt[2 * DH:WROWS].astype(_BF16)
            qt_v[:, T * 128:(T + 1) * 128] = _u32(qtile)
            for slot in range(HB):
                bcast_rows(qtile[slot * DH:(slot + 1) * DH].astype(_F32), slot, T)
    kap_v[...] = jnp.broadcast_to(jnp.max(kmax, axis=1, keepdims=True), (DH, 128))
    cp_wu.wait()
    wup_v[...] = _u32(wu_v[...])
    for slot in range(HB):
        for T in range(NT):
            shift_rows(_bf(qt_v[slot * 8:(slot + 1) * 8, T * 128:(T + 1) * 128]).astype(_F32),
                       slot, T)

    def finish(hrow, u, l, acc):
        lt = jnp.sum(l, axis=0, keepdims=True)
        r0 = hrow * DH if isinstance(hrow, int) else pl.multiple_of(hrow * DH, DH)
        ot_v[pl.ds(r0, DH), u * TQ:(u + 1) * TQ] = (acc / lt).astype(_BF16)
        return lt

    def deferred_pv(j, acc):
        c = NC - 2 + j
        o = jnp.dot(_bf(vt_v[:, c * CK:(c + 1) * CK]), _bf(pc_v[j]),
                    preferred_element_type=_F32)
        return (acc_v[...] if acc is None else acc) + o

    def body(j, carry):
        lmin, lmax = carry
        h0 = j * HB
        zi = z_v[...]
        never = zi != 0
        never2 = _rep(zi) != 0
        zf = pltpu.bitcast(zi, _F32)
        zf_acc = _rep(jnp.concatenate([zf] * 4, axis=1))
        zf_gate = _rep(zf, RM // 8)
        P = {}
        SC = {}
        G = {}
        L = [None] * NW
        ACC = [None] * NW
        prev = {}
        n_ffn = [0]

        def pv_pos(w, c):
            return w * NMS + LASTS[c] + LAG

        def q_aug(w):
            hb, u = divmod(w, NQ)
            lo = qt_v[pl.ds(pl.multiple_of((h0 + hb) * 8, 8), 8), u * TQ:(u + 1) * TQ]
            hi = qhi_bufs[hb][:, u * TQ:(u + 1) * TQ]
            return _bf(jnp.concatenate([lo, hi], axis=0))

        def consume(w, c, g, s0, s1):
            p0 = jnp.exp2(s0)
            p1 = jnp.exp2(s1)
            t = p0 + p1
            L[w] = t if L[w] is None else L[w] + t
            P[(w, c, g)] = (p0, p1)

        def mxu_scores(w, i0, i1):
            s = jnp.dot(_bf(kp_v[i0 * 8:i1 * 8, :]), q_aug(w), preferred_element_type=_F32)
            for i in range(i0, i1):
                o = (i - i0) * 16
                consume(w, *MSL[i], s[o:o + 8], s[o + 8:o + 16])
                SC[w * NMS + i] = s[o:o + 8, 0:128]

        def vpu_scores(w, c, g, dep):
            hb, u = divmod(w, NQ)
            qb_ref = qb_bufs[hb]
            kb0 = (VB[c] + g) * DH
            serial = w == 0 and c == 0 and g == 1
            res = []
            for t in range(4):
                base = (u * 4 + t) * QR
                cols = slice(t * 128, (t + 1) * 128)
                if serial:
                    halves = []
                    for gg in range(2):
                        a = qb_ref[base + DH]
                        if dep is not None:
                            a = jnp.where(never, dep[8:16], a)
                        for d in range(DH):
                            a = a + kb_v[kb0 + d, gg * 8:(gg + 1) * 8, cols] * qb_ref[base + d]
                        halves.append(a)
                        dep = _rep(a)
                    res.append(jnp.concatenate(halves, axis=0))
                else:
                    a = _rep(qb_ref[base + DH])
                    if dep is not None:
                        a = jnp.where(never2, dep, a)
                    for d in range(DH):
                        a = a + kb_v[kb0 + d, :, cols] * _rep(qb_ref[base + d])
                    res.append(a)
                    dep = a
            s = jnp.concatenate(res, axis=1)
            consume(w, c, g, s[0:8], s[8:16])
            return dep

        def p_tile(w, c, anchor=None):
            dep = None if anchor is None else _rep(anchor)
            for g in range(NVS[c] - 1, -1, -1):
                dep = vpu_scores(w, c, g, dep)
            ps = []
            for g in range(8):
                ps += list(P.pop((w, c, g)))
            return jnp.concatenate(ps, axis=0).astype(_BF16)

        def refill(w, k, anchor):
            hb, u = divmod(w, NQ)
            T = u * 4 + k
            hn = jnp.minimum(h0 + hb + HB, H - 1)
            qp = qt_v[pl.ds(pl.multiple_of(hn * 8, 8), 8), T * 128:(T + 1) * 128]
            q = _bf(jnp.where(never, _u32(anchor), qp)).astype(_F32)
            bcast_rows(q, hb, T)
            shift_rows(q, hb, T)

        def ffn_matmul():
            hb, k = divmod(n_ffn[0], 2 * NF)
            f, is_up = divmod(k, 2)
            n_ffn[0] += 1
            x = x_v[pl.ds(pl.multiple_of((h0 + hb) * RM, RM), RM), :]
            wref = wup_v if is_up else wgp_v
            y = jnp.dot(x, _bf(wref[:, f * 128:(f + 1) * 128]), preferred_element_type=_F32)
            if not is_up:
                G[f] = y + zf_gate
            else:
                gh = 0.5 * G.pop(f)
                gu = gh * y
                r0 = pl.multiple_of((h0 + hb) * (RM // 2), RM // 2)
                h_v[pl.ds(r0, RM // 2), f * 128:(f + 1) * 128] = _u32(
                    (gu + gu * jnp.tanh(gh)).astype(_BF16))

        def do_pv(w, c):
            if w < 0:
                prev["acc"] = deferred_pv(c - (NC - 2), prev.get("acc"))
                if c == NC - 1:
                    prev["lt"] = finish(h0, NQ - 1, l_v[...], prev["acc"])
            else:
                anchor = SC[pv_pos(w, c) - ANCHOR_LAST] if c == NC - 1 else None
                o = jnp.dot(_bf(vt_v[:, c * CK:(c + 1) * CK]), p_tile(w, c, anchor),
                            preferred_element_type=_F32)
                ACC[w] = (o + zf_acc) if ACC[w] is None else ACC[w] + o
                if c == NC - 1:
                    L[w] = finish(h0 + w // NQ + 1, w % NQ, L[w], ACC[w])
                if c in REFILL_AT and w > 0:
                    refill(w - 1, REFILL_AT.index(c), SC[pv_pos(w, c) - LAG])
            for _ in range(FFN_AFTER.get(c, 0)):
                ffn_matmul()

        tot = NW * NMS
        pv_at = {pv_pos(w, c): (w, c) for w in range(-1, NW) for c in range(NC)
                 if 0 <= pv_pos(w, c) < tot}
        start = 0
        for gi in range(tot):
            w, i = divmod(gi, NMS)
            if gi in pv_at or i == NMS - 1:
                mxu_scores(w, start, i + 1)
                start = (i + 1) % NMS
            if gi in pv_at:
                do_pv(*pv_at[gi])
        assert n_ffn[0] == HB * 2 * NF and not G
        for k in range(2):
            c = NC - 2 + k
            anchor = SC[pv_pos(NW - 1, c) - LAG - ANCHOR_CARRY]
            pc_v[k] = _u32(p_tile(NW - 1, c, anchor))
        assert not P
        acc_v[...] = ACC[NW - 1]
        l_v[...] = L[NW - 1]
        for k in range(4):
            refill(NW - 1, k, SC[tot - ANCHOR_TAIL_REFILL[k]])
        for lt in [prev["lt"]] + L[:NW - 1]:
            lmin = jnp.minimum(lmin, lt)
            lmax = jnp.maximum(lmax, lt)
        return lmin, lmax

    lmin, lmax = lax.fori_loop(
        0, H // HB, body, (jnp.full((1, TQ), L_HI, _F32), jnp.full((1, TQ), L_LO, _F32)))
    lt = finish(H, NQ - 1, l_v[...], deferred_pv(1, deferred_pv(0, None)))
    lmin = jnp.minimum(lmin, lt)
    lmax = jnp.maximum(lmax, lt)
    safe = jnp.logical_and(lmin >= L_LO, lmax <= L_HI)
    n_unsafe = jnp.sum(jnp.where(safe, 0.0, 1.0))

    @pl.when(n_unsafe > 0.0)
    def _():
        def item(i, carry):
            h = i // NQ
            c0 = pl.multiple_of((i % NQ) * TQ, TQ)
            qt = _bf(qt_v[pl.ds(pl.multiple_of(h * 8, 8), 8), pl.ds(c0, TQ)])

            def scores(c, m8):
                r0 = pl.multiple_of(c * CK, CK)
                s = jnp.dot(kn_v[pl.ds(r0, CK), :], qt, preferred_element_type=_F32)
                s_v[pl.ds(r0, CK), :] = s
                return jnp.maximum(m8, jnp.max(s.reshape(CK // 8, 8, TQ), axis=0))

            m8 = lax.fori_loop(0, NC, scores, jnp.full((8, TQ), -jnp.inf, _F32))
            m = jnp.max(m8, axis=0, keepdims=True)

            def pv(c, st):
                l, acc = st
                r0 = pl.multiple_of(c * CK, CK)
                p = jnp.exp2(s_v[pl.ds(r0, CK), :] - m)
                l = l + jnp.sum(p.reshape(CK // 8, 8, TQ), axis=0)
                acc = acc + jnp.dot(_bf(vt_v[:, pl.ds(r0, CK)]), p.astype(_BF16),
                                    preferred_element_type=_F32)
                return l, acc

            l, acc = lax.fori_loop(0, NC, pv, (jnp.zeros((8, TQ), _F32),
                                               jnp.zeros((DH, TQ), _F32)))
            lt = jnp.sum(l, axis=0, keepdims=True)
            ot_v[pl.ds(pl.multiple_of((h + 1) * DH, DH), DH), pl.ds(c0, TQ)] = (
                (acc / lt).astype(_BF16))
            return carry

        lax.fori_loop(0, H * NQ, item, 0)

    for cp in (cp_gw, cp_wd, cp_wo):
        cp.wait()

    def out_copy(t):
        r0 = t * TM if isinstance(t, int) else pl.multiple_of(t * TM, TM)
        return pltpu.make_async_copy(out_v.at[pl.ds(r0, TM)], out_hbm.at[pl.ds(r0, TM)],
                                     out_sems.at[t])

    def final(t, carry):
        r0 = pl.multiple_of(t * TM, TM)
        xf = x_v[pl.ds(r0, TM), :].astype(_F32)
        gw = gw_v[...].astype(_F32)
        z = xf[:, 0:128] * gw[0:1, :]
        for j in range(1, D // 128):
            z = z + xf[:, j * 128:(j + 1) * 128] * gw[j:j + 1, :]
        gate = jax.nn.sigmoid(jnp.sum(z, axis=-1, keepdims=True))
        hh = _bf(h_v[pl.ds(pl.multiple_of(t * (TM // 2), TM // 2), TM // 2), :])
        b = jnp.dot(hh, wd_v[...], preferred_element_type=_F32)
        ot = ot_v[DH:(H + 1) * DH, pl.ds(r0, TM)]
        a = lax.dot_general(ot, wo_v[...], (((0,), (0,)), ((), ())),
                            preferred_element_type=_F32)
        out_v[pl.ds(r0, TM), :] = (gate * a + (1.0 - gate) * b).astype(_BF16)
        out_copy(t).start()
        return carry

    lax.fori_loop(0, NM, final, 0)

    for t in range(NM):
        out_copy(t).wait()


@jax.jit
def pallas_gated_mix__grouped_kv_mqa__swiglu_ffn__prompt_kernel(
    A_x: jax.Array,
    A_wq: jax.Array,
    A_wk: jax.Array,
    A_wv: jax.Array,
    A_wo: jax.Array,
    B_x: jax.Array,
    B_w_gate: jax.Array,
    B_w_up: jax.Array,
    B_w_down: jax.Array,
    gate_w: jax.Array,
):
    del B_x
    any_spec = pl.BlockSpec(memory_space=pl.ANY)
    out = pl.pallas_call(
        _kernel,
        out_shape=jax.ShapeDtypeStruct((S, D), _BF16),
        in_specs=[any_spec] * 9,
        out_specs=any_spec,
        scratch_shapes=[
            pltpu.VMEM((S, D), _BF16),
            pltpu.VMEM((D, H * DH), _BF16),
            pltpu.VMEM((H * DH, D), _BF16),
            pltpu.VMEM((D, F), _BF16),
            pltpu.VMEM((D, F), _BF16),
            pltpu.VMEM((F, D), _BF16),
            pltpu.VMEM((D // 128, 128), _BF16),
            pltpu.VMEM((D // 2, F), _U32),
            pltpu.VMEM((D // 2, F), _U32),
            pltpu.VMEM((WROWS, D), _BF16),
            pltpu.VMEM((H * DH // 2, S), _U32),
            pltpu.VMEM((NMS * 8, KA), _U32),
            pltpu.VMEM((S, DH), _BF16),
            pltpu.VMEM((VB[NC] * DH, 16, TQ), _F32),
            pltpu.VMEM((DH // 2, S), _U32),
            pltpu.VMEM((DH, 128), _F32),
            pltpu.VMEM((8, 128), jnp.int32),
            pltpu.VMEM((2, CK // 2, TQ), _U32),
            pltpu.VMEM((DH, TQ), _F32),
            pltpu.VMEM((8, TQ), _F32),
            pltpu.VMEM(((H + 1) * DH, S), _BF16),
            pltpu.VMEM((S // 2, F), _U32),
            pltpu.VMEM((S, TQ), _F32),
            pltpu.VMEM((S, D), _BF16),
            pltpu.SemaphoreType.DMA((NX + 8,)),
            pltpu.SemaphoreType.DMA((NM,)),
        ] + [pltpu.VMEM((NT * QR, 8, 128), _F32)] * HB + [pltpu.VMEM((8, S), _U32)] * HB,
        compiler_params=pltpu.CompilerParams(vmem_limit_bytes=100 * 1024 * 1024),
    )(A_x.reshape(S, D), A_wq, A_wk.T, A_wv.T, A_wo, B_w_gate, B_w_up, B_w_down,
      gate_w.reshape(D // 128, 128))
    return out.reshape(1, S, D)
```

```python
import math

import jax
import jax.numpy as jnp
from jax import lax
import jax.experimental.pallas as pl
import jax.experimental.pallas.tpu as pltpu

S, D, H, DH, F = 2048, 512, 32, 16, 1792
TQ = 512
NQ = S // TQ
NT = S // 128
CK = 128
NC = S // CK
TCS = (256, 512, 768, 512)
NX = len(TCS)
TX = [sum(TCS[:c]) for c in range(NX + 1)]
TM = 512
NM = S // TM
TN = 256
NN = D // TN
RM = S // H
NF = F // 128
WROWS = H * DH + 2 * DH
KA = 2 * DH
QR = DH + 1
KSCALE = (DH ** -0.5) * math.log2(math.e)

NVS = [2 if c in (0, 3, 8) else 1 for c in range(NC)]
VB = [sum(NVS[:c]) for c in range(NC + 1)]
MSL = [(c, g) for c in range(NC) for g in range(7, NVS[c] - 1, -1)]
NMS = len(MSL)
LASTS = [max(i for i, cg in enumerate(MSL) if cg[0] == c) for c in range(NC)]
HB = 4
NW = HB * NQ
LAG = 10
FFN_AFTER = {2: 2, 7: 2, 15: 3}
REFILL_AT = (1, 5, 9, 13)
ANCHOR_LAST = 16
ANCHOR_CARRY = 21
ANCHOR_TAIL_REFILL = (7, 6, 5, 4)
WG_REPACK = (0, 8, NF)

L_LO = 2.0 ** -50
L_HI = 2.0 ** 60

_F32 = jnp.float32
_BF16 = jnp.bfloat16
_U32 = jnp.uint32


def _bf(v):
    return pltpu.bitcast(v, _BF16)


def _u32(v):
    return pltpu.bitcast(v, _U32)


def _rep(v, n=2):
    return jnp.concatenate([v] * n, axis=0)


def _kernel(x_hbm, wq_hbm, wkt_hbm, wvt_hbm, wo_hbm, wg_hbm, wu_hbm, wd_hbm, gw_hbm,
            out_hbm,
            x_v, wq_v, wo_v, wg_v, wu_v, wd_v, gw_v, wgp_v, wup_v, wt_v, qt_v, kp_v, kn_v,
            kb_v, vt_v, kap_v, z_v, pc_v, acc_v, l_v, ot_v, h_v, s_v, out_v,
            in_sems, out_sems, *bufs):
    qb_bufs, qhi_bufs = bufs[:HB], bufs[HB:]

    def load(i, src, dst):
        return pltpu.make_async_copy(src, dst, in_sems.at[i])

    cp_x = [load(c, x_hbm.at[pl.ds(TX[c], TCS[c])], x_v.at[pl.ds(TX[c], TCS[c])])
            for c in range(NX)]
    cp_wq = load(NX, wq_hbm, wq_v)
    cp_wk = load(NX + 1, wkt_hbm, wt_v.at[pl.ds(0, DH)])
    cp_wv = load(NX + 2, wvt_hbm, wt_v.at[pl.ds(DH, DH)])
    cp_wg = load(NX + 3, wg_hbm, wg_v)
    cp_wu = load(NX + 4, wu_hbm, wu_v)
    cp_gw = load(NX + 5, gw_hbm, gw_v)
    cp_wd = load(NX + 6, wd_hbm, wd_v)
    cp_wo = load(NX + 7, wo_hbm, wo_v)
    for cp in (cp_wq, cp_x[0], cp_wk, cp_wv, *cp_x[1:NX - 1], cp_wg, cp_x[NX - 1], cp_wu, cp_gw,
               cp_wd, cp_wo):
        cp.start()

    z_v[...] = jnp.zeros((8, 128), jnp.int32)
    pc_v[...] = jnp.zeros((2, CK // 2, TQ), _U32)
    acc_v[...] = jnp.zeros((DH, TQ), _F32)
    l_v[...] = jnp.ones((8, TQ), _F32)
    cp_wq.wait()
    wt_v[2 * DH:WROWS, :] = wq_v[...].T
    cp_wk.wait()
    cp_wv.wait()

    def bcast_rows(q, slot, T):
        for d in range(DH):
            qb_bufs[slot][T * QR + d] = jnp.broadcast_to(q[d:d + 1, :], (8, 128))

    def shift_rows(q, slot, T):
        w = (jnp.abs(q) * kap_v[...]).astype(_BF16)
        qhi_bufs[slot][:, T * 128:(T + 1) * 128] = _u32(w)
        nb = -jnp.sum(w.astype(_F32), axis=0, keepdims=True)
        qb_bufs[slot][T * QR + DH] = jnp.broadcast_to(nb, (8, 128))

    def store_k(kt, T):
        kaug = jnp.concatenate([kt, jnp.full((DH, 128), -1.0, _F32)], axis=0).T
        kn_v[T * 128:(T + 1) * 128, :] = kaug[:, 0:DH].astype(_BF16)
        for i, (cc, g) in enumerate(MSL):
            if cc == T:
                kp_v[i * 8:(i + 1) * 8, :] = _u32(kaug[g * 16:(g + 1) * 16].astype(_BF16))
        for g in range(NVS[T]):
            for d in range(DH):
                kb_v[(VB[T] + g) * DH + d] = jnp.broadcast_to(
                    kaug[g * 16:(g + 1) * 16, d:d + 1], (16, TQ))

    kmax = None
    pending = []
    for c in range(NX):
        cp_x[c].wait()
        if c == NX - 1:
            cp_wg.wait()
        while pending:
            store_k(*pending.pop(0))
        r = lax.dot_general(wt_v[...], x_v[TX[c]:TX[c + 1], :],
                            (((1,), (1,)), ((), ())), preferred_element_type=_F32)
        for t in range(TCS[c] // 128):
            T = TX[c] // 128 + t
            rt = r[:, t * 128:(t + 1) * 128]
            kt = (rt[0:DH] * KSCALE).astype(_BF16).astype(_F32)
            a = jnp.abs(kt)
            kmax = a if kmax is None else jnp.maximum(kmax, a)
            vt_v[:, T * 128:(T + 1) * 128] = _u32(rt[DH:2 * DH].astype(_BF16))
            if t == TCS[c] // 128 - 1 and c < NX - 1:
                pending.append((kt, T))
            else:
                store_k(kt, T)
            if c == NX - 1 and t < len(WG_REPACK) - 1:
                f0, f1 = WG_REPACK[t], WG_REPACK[t + 1]
                for f in range(f0, f1):
                    row = (((f - f0) * WROWS) // (f1 - f0)) // 8 * 8
                    wgp_v[:, f * 128:(f + 1) * 128] = jnp.where(
                        _rep(z_v[...], D // 16) != 0, _rep(_u32(rt[row:row + 8]), D // 16),
                        _u32(wg_v[:, f * 128:(f + 1) * 128]))
            qtile = rt[2 * DH:WROWS].astype(_BF16)
            qt_v[:, T * 128:(T + 1) * 128] = _u32(qtile)
            for slot in range(HB):
                bcast_rows(qtile[slot * DH:(slot + 1) * DH].astype(_F32), slot, T)
    kap_v[...] = jnp.broadcast_to(jnp.max(kmax, axis=1, keepdims=True), (DH, 128))
    for slot in range(HB):
        for T in range(NT):
            shift_rows(_bf(qt_v[slot * 8:(slot + 1) * 8, T * 128:(T + 1) * 128]).astype(_F32),
                       slot, T)
    cp_wu.wait()
    wup_v[...] = _u32(wu_v[...])

    def finish(hrow, u, l, acc):
        lt = jnp.sum(l, axis=0, keepdims=True)
        r0 = hrow * DH if isinstance(hrow, int) else pl.multiple_of(hrow * DH, DH)
        ot_v[pl.ds(r0, DH), u * TQ:(u + 1) * TQ] = (acc / lt).astype(_BF16)
        return lt

    def deferred_pv(j, acc):
        c = NC - 2 + j
        o = jnp.dot(_bf(vt_v[:, c * CK:(c + 1) * CK]), _bf(pc_v[j]),
                    preferred_element_type=_F32)
        return (acc_v[...] if acc is None else acc) + o

    def body(j, carry):
        lmin, lmax = carry
        h0 = j * HB
        zi = z_v[...]
        never = zi != 0
        never2 = _rep(zi) != 0
        zf = pltpu.bitcast(zi, _F32)
        zf_acc = _rep(jnp.concatenate([zf] * 4, axis=1))
        zf_gate = _rep(zf, RM // 8)
        P = {}
        SC = {}
        G = {}
        L = [None] * NW
        ACC = [None] * NW
        prev = {}
        n_ffn = [0]

        def pv_pos(w, c):
            return w * NMS + LASTS[c] + LAG

        def q_aug(w):
            hb, u = divmod(w, NQ)
            lo = qt_v[pl.ds(pl.multiple_of((h0 + hb) * 8, 8), 8), u * TQ:(u + 1) * TQ]
            hi = qhi_bufs[hb][:, u * TQ:(u + 1) * TQ]
            return _bf(jnp.concatenate([lo, hi], axis=0))

        def consume(w, c, g, s0, s1):
            p0 = jnp.exp2(s0)
            p1 = jnp.exp2(s1)
            t = p0 + p1
            L[w] = t if L[w] is None else L[w] + t
            P[(w, c, g)] = (p0, p1)

        def mxu_scores(w, i0, i1):
            s = jnp.dot(_bf(kp_v[i0 * 8:i1 * 8, :]), q_aug(w), preferred_element_type=_F32)
            for i in range(i0, i1):
                o = (i - i0) * 16
                consume(w, *MSL[i], s[o:o + 8], s[o + 8:o + 16])
                SC[w * NMS + i] = s[o:o + 8, 0:128]

        def vpu_scores(w, c, g, dep):
            hb, u = divmod(w, NQ)
            qb_ref = qb_bufs[hb]
            kb0 = (VB[c] + g) * DH
            serial = w == 0 and c == 0 and g == 1
            res = []
            for t in range(4):
                base = (u * 4 + t) * QR
                cols = slice(t * 128, (t + 1) * 128)
                if serial:
                    halves = []
                    for gg in range(2):
                        a = qb_ref[base + DH]
                        if dep is not None:
                            a = jnp.where(never, dep[8:16], a)
                        for d in range(DH):
                            a = a + kb_v[kb0 + d, gg * 8:(gg + 1) * 8, cols] * qb_ref[base + d]
                        halves.append(a)
                        dep = _rep(a)
                    res.append(jnp.concatenate(halves, axis=0))
                else:
                    a = _rep(qb_ref[base + DH])
                    if dep is not None:
                        a = jnp.where(never2, dep, a)
                    for d in range(DH):
                        a = a + kb_v[kb0 + d, :, cols] * _rep(qb_ref[base + d])
                    res.append(a)
                    dep = a
            s = jnp.concatenate(res, axis=1)
            consume(w, c, g, s[0:8], s[8:16])
            return dep

        def p_tile(w, c, anchor=None):
            dep = None if anchor is None else _rep(anchor)
            for g in range(NVS[c] - 1, -1, -1):
                dep = vpu_scores(w, c, g, dep)
            ps = []
            for g in range(8):
                ps += list(P.pop((w, c, g)))
            return jnp.concatenate(ps, axis=0).astype(_BF16)

        def refill(w, k, anchor):
            hb, u = divmod(w, NQ)
            T = u * 4 + k
            hn = jnp.minimum(h0 + hb + HB, H - 1)
            qp = qt_v[pl.ds(pl.multiple_of(hn * 8, 8), 8), T * 128:(T + 1) * 128]
            q = _bf(jnp.where(never, _u32(anchor), qp)).astype(_F32)
            bcast_rows(q, hb, T)
            shift_rows(q, hb, T)

        def ffn_matmul():
            hb, k = divmod(n_ffn[0], 2 * NF)
            f, is_up = divmod(k, 2)
            n_ffn[0] += 1
            x = x_v[pl.ds(pl.multiple_of((h0 + hb) * RM, RM), RM), :]
            wref = wup_v if is_up else wgp_v
            y = jnp.dot(x, _bf(wref[:, f * 128:(f + 1) * 128]), preferred_element_type=_F32)
            if not is_up:
                G[f] = y + zf_gate
            else:
                gh = 0.5 * G.pop(f)
                gu = gh * y
                r0 = pl.multiple_of((h0 + hb) * (RM // 2), RM // 2)
                h_v[pl.ds(r0, RM // 2), f * 128:(f + 1) * 128] = _u32(
                    (gu + gu * jnp.tanh(gh)).astype(_BF16))

        def do_pv(w, c):
            if w < 0:
                prev["acc"] = deferred_pv(c - (NC - 2), prev.get("acc"))
                if c == NC - 1:
                    prev["lt"] = finish(h0, NQ - 1, l_v[...], prev["acc"])
            else:
                anchor = SC[pv_pos(w, c) - ANCHOR_LAST] if c == NC - 1 else None
                o = jnp.dot(_bf(vt_v[:, c * CK:(c + 1) * CK]), p_tile(w, c, anchor),
                            preferred_element_type=_F32)
                ACC[w] = (o + zf_acc) if ACC[w] is None else ACC[w] + o
                if c == NC - 1:
                    L[w] = finish(h0 + w // NQ + 1, w % NQ, L[w], ACC[w])
                if c in REFILL_AT and w > 0:
                    refill(w - 1, REFILL_AT.index(c), SC[pv_pos(w, c) - LAG])
            for _ in range(FFN_AFTER.get(c, 0)):
                ffn_matmul()

        tot = NW * NMS
        pv_at = {pv_pos(w, c): (w, c) for w in range(-1, NW) for c in range(NC)
                 if 0 <= pv_pos(w, c) < tot}
        start = 0
        for gi in range(tot):
            w, i = divmod(gi, NMS)
            if gi in pv_at or i == NMS - 1:
                mxu_scores(w, start, i + 1)
                start = (i + 1) % NMS
            if gi in pv_at:
                do_pv(*pv_at[gi])
        assert n_ffn[0] == HB * 2 * NF and not G
        for k in range(2):
            c = NC - 2 + k
            anchor = SC[pv_pos(NW - 1, c) - LAG - ANCHOR_CARRY]
            pc_v[k] = _u32(p_tile(NW - 1, c, anchor))
        assert not P
        acc_v[...] = ACC[NW - 1]
        l_v[...] = L[NW - 1]
        for k in range(4):
            refill(NW - 1, k, SC[tot - ANCHOR_TAIL_REFILL[k]])
        for lt in [prev["lt"]] + L[:NW - 1]:
            lmin = jnp.minimum(lmin, lt)
            lmax = jnp.maximum(lmax, lt)
        return lmin, lmax

    lmin, lmax = lax.fori_loop(
        0, H // HB, body, (jnp.full((1, TQ), L_HI, _F32), jnp.full((1, TQ), L_LO, _F32)))
    lt = finish(H, NQ - 1, l_v[...], deferred_pv(1, deferred_pv(0, None)))
    lmin = jnp.minimum(lmin, lt)
    lmax = jnp.maximum(lmax, lt)
    safe = jnp.logical_and(lmin >= L_LO, lmax <= L_HI)
    n_unsafe = jnp.sum(jnp.where(safe, 0.0, 1.0))

    @pl.when(n_unsafe > 0.0)
    def _():
        def item(i, carry):
            h = i // NQ
            c0 = pl.multiple_of((i % NQ) * TQ, TQ)
            qt = _bf(qt_v[pl.ds(pl.multiple_of(h * 8, 8), 8), pl.ds(c0, TQ)])

            def scores(c, m8):
                r0 = pl.multiple_of(c * CK, CK)
                s = jnp.dot(kn_v[pl.ds(r0, CK), :], qt, preferred_element_type=_F32)
                s_v[pl.ds(r0, CK), :] = s
                return jnp.maximum(m8, jnp.max(s.reshape(CK // 8, 8, TQ), axis=0))

            m8 = lax.fori_loop(0, NC, scores, jnp.full((8, TQ), -jnp.inf, _F32))
            m = jnp.max(m8, axis=0, keepdims=True)

            def pv(c, st):
                l, acc = st
                r0 = pl.multiple_of(c * CK, CK)
                p = jnp.exp2(s_v[pl.ds(r0, CK), :] - m)
                l = l + jnp.sum(p.reshape(CK // 8, 8, TQ), axis=0)
                acc = acc + jnp.dot(_bf(vt_v[:, pl.ds(r0, CK)]), p.astype(_BF16),
                                    preferred_element_type=_F32)
                return l, acc

            l, acc = lax.fori_loop(0, NC, pv, (jnp.zeros((8, TQ), _F32),
                                               jnp.zeros((DH, TQ), _F32)))
            lt = jnp.sum(l, axis=0, keepdims=True)
            ot_v[pl.ds(pl.multiple_of((h + 1) * DH, DH), DH), pl.ds(c0, TQ)] = (
                (acc / lt).astype(_BF16))
            return carry

        lax.fori_loop(0, H * NQ, item, 0)

    for cp in (cp_gw, cp_wd, cp_wo):
        cp.wait()

    def out_copy(t, n):
        r0 = t * TM if isinstance(t, int) else pl.multiple_of(t * TM, TM)
        blk = (pl.ds(r0, TM), pl.ds(n * TN, TN))
        return pltpu.make_async_copy(out_v.at[blk], out_hbm.at[blk], out_sems.at[NN * t + n])

    def final(t, carry):
        r0 = pl.multiple_of(t * TM, TM)
        xf = x_v[pl.ds(r0, TM), :].astype(_F32)
        gw = gw_v[...].astype(_F32)
        z = xf[:, 0:128] * gw[0:1, :]
        for j in range(1, D // 128):
            z = z + xf[:, j * 128:(j + 1) * 128] * gw[j:j + 1, :]
        gate = jax.nn.sigmoid(jnp.sum(z, axis=-1, keepdims=True))
        hh = _bf(h_v[pl.ds(pl.multiple_of(t * (TM // 2), TM // 2), TM // 2), :])
        ot = ot_v[DH:(H + 1) * DH, pl.ds(r0, TM)]
        for n in range(NN):
            cols = slice(n * TN, (n + 1) * TN)
            b = jnp.dot(hh, wd_v[:, cols], preferred_element_type=_F32)
            a = lax.dot_general(ot, wo_v[:, cols], (((0,), (0,)), ((), ())),
                                preferred_element_type=_F32)
            out_v[pl.ds(r0, TM), cols] = (gate * a + (1.0 - gate) * b).astype(_BF16)
            out_copy(t, n).start()
        return carry

    lax.fori_loop(0, NM, final, 0)

    for t in range(NM):
        for n in range(NN):
            out_copy(t, n).wait()


@jax.jit
def pallas_gated_mix__grouped_kv_mqa__swiglu_ffn__prompt_kernel(
    A_x: jax.Array,
    A_wq: jax.Array,
    A_wk: jax.Array,
    A_wv: jax.Array,
    A_wo: jax.Array,
    B_x: jax.Array,
    B_w_gate: jax.Array,
    B_w_up: jax.Array,
    B_w_down: jax.Array,
    gate_w: jax.Array,
):
    del B_x
    any_spec = pl.BlockSpec(memory_space=pl.ANY)
    out = pl.pallas_call(
        _kernel,
        out_shape=jax.ShapeDtypeStruct((S, D), _BF16),
        in_specs=[any_spec] * 9,
        out_specs=any_spec,
        scratch_shapes=[
            pltpu.VMEM((S, D), _BF16),
            pltpu.VMEM((D, H * DH), _BF16),
            pltpu.VMEM((H * DH, D), _BF16),
            pltpu.VMEM((D, F), _BF16),
            pltpu.VMEM((D, F), _BF16),
            pltpu.VMEM((F, D), _BF16),
            pltpu.VMEM((D // 128, 128), _BF16),
            pltpu.VMEM((D // 2, F), _U32),
            pltpu.VMEM((D // 2, F), _U32),
            pltpu.VMEM((WROWS, D), _BF16),
            pltpu.VMEM((H * DH // 2, S), _U32),
            pltpu.VMEM((NMS * 8, KA), _U32),
            pltpu.VMEM((S, DH), _BF16),
            pltpu.VMEM((VB[NC] * DH, 16, TQ), _F32),
            pltpu.VMEM((DH // 2, S), _U32),
            pltpu.VMEM((DH, 128), _F32),
            pltpu.VMEM((8, 128), jnp.int32),
            pltpu.VMEM((2, CK // 2, TQ), _U32),
            pltpu.VMEM((DH, TQ), _F32),
            pltpu.VMEM((8, TQ), _F32),
            pltpu.VMEM(((H + 1) * DH, S), _BF16),
            pltpu.VMEM((S // 2, F), _U32),
            pltpu.VMEM((S, TQ), _F32),
            pltpu.VMEM((S, D), _BF16),
            pltpu.SemaphoreType.DMA((NX + 8,)),
            pltpu.SemaphoreType.DMA((NN * NM,)),
        ] + [pltpu.VMEM((NT * QR, 8, 128), _F32)] * HB + [pltpu.VMEM((8, S), _U32)] * HB,
        compiler_params=pltpu.CompilerParams(vmem_limit_bytes=100 * 1024 * 1024),
    )(A_x.reshape(S, D), A_wq, A_wk.T, A_wv.T, A_wo, B_w_gate, B_w_up, B_w_down,
      gate_w.reshape(D // 128, 128))
    return out.reshape(1, S, D)
```
